```python
import os as _os
_os.environ.setdefault("JAX_PLATFORMS", "cpu")
import jax
import jax.numpy as jnp

def _softmax(x, axis=-1):
    return jax.nn.softmax(x, axis=axis)
def _gelu(x):
    return jax.nn.gelu(x, approximate=True)
def _silu(x):
    return jax.nn.silu(x)
def _sigmoid(x):
    return jax.nn.sigmoid(x)
def _layernorm(x, axis=-1, eps=1e-5):
    m = jnp.mean(x, axis=axis, keepdims=True)
    v = jnp.var(x, axis=axis, keepdims=True)
    return (x - m) / jnp.sqrt(v + eps)
def _scatter_add(tgt, idx, src, axis=0):
    return tgt.at[idx].add(src)
def _segment_sum(src, seg, n):
    return jax.ops.segment_sum(src, seg, n)
class _Rng:
    def __init__(self, key):
        self._k = key
    def _next(self):
        self._k, sub = jax.random.split(self._k)
        return sub
    def normal(self, shape):
        return jax.random.normal(self._next(), shape, dtype=jnp.bfloat16)
    def randint(self, lo, hi, shape):
        return jax.random.randint(self._next(), shape, lo, hi, dtype=jnp.int32)
    def uniform(self, shape, lo=0.0, hi=1.0):
        return jax.random.uniform(self._next(), shape, jnp.bfloat16, lo, hi)
    def permutation(self, n):
        return jax.random.permutation(self._next(), n)


kernel_name = 'concat_heads__sliding_block__ssm_conv_s4__prompt'

def setup_inputs():
    _rng = _Rng(jax.random.key(int.from_bytes(__import__("os").urandom(4), "little")))
    _w = (lambda a: (lambda t: t.astype(jnp.bfloat16) if jnp.issubdtype(t.dtype, jnp.floating) else t)(jnp.asarray(a)))
    def _A_setup():
        B, S, D = 1, 2048, 512
        return {
            "x": _w((lambda *s: _rng.normal(s) * 0.2)(B, S, D)),
            "wqkv": _w((lambda *s: _rng.normal(s) * 0.2)(D, 3 * D)),
            "wo": _w((lambda *s: _rng.normal(s) * 0.05)(D, D)),
        }
    _A_in = _A_setup()

    def _B_setup():
        B, L, D, N = 1, 2048, 512, 128
        A_re = -jnp.exp((lambda *s: _rng.normal(s) * 0.8)(D, N))
        A_im = jnp.pi * (lambda *s: _rng.normal(s) * 0.8)(D, N)
        B_re = (lambda *s: _rng.normal(s) * 0.8)(D, N)
        B_im = (lambda *s: _rng.normal(s) * 0.8)(D, N)
        C_re = (lambda *s: _rng.normal(s) * 0.8)(D, N)
        C_im = (lambda *s: _rng.normal(s) * 0.8)(D, N)
        log_dt = (lambda *s: _rng.normal(s) * 0.8)(D) * 0.5 - 4.0
        Dskip = (lambda *s: _rng.normal(s) * 0.05)(D)
        return {
            "u": _w((lambda *s: _rng.normal(s) * 0.05)(B, L, D)),
            "A_re": _w(A_re),
            "A_im": _w(A_im),
            "B_re": _w(B_re),
            "B_im": _w(B_im),
            "C_re": _w(C_re),
            "C_im": _w(C_im),
            "log_dt": _w(log_dt),
            "Dskip": _w(Dskip),
        }
    _B_in = _B_setup()

    return {
        "A_x": _A_in["x"],
        "A_wqkv": _A_in["wqkv"],
        "A_wo": _A_in["wo"],
        "B_u": _B_in["u"],
        "B_A_re": _B_in["A_re"],
        "B_A_im": _B_in["A_im"],
        "B_B_re": _B_in["B_re"],
        "B_B_im": _B_in["B_im"],
        "B_C_re": _B_in["C_re"],
        "B_C_im": _B_in["C_im"],
        "B_log_dt": _B_in["log_dt"],
        "B_Dskip": _B_in["Dskip"],
    }

def reference(A_x, A_wqkv, A_wo, B_u, B_A_re, B_A_im, B_B_re, B_B_im, B_C_re, B_C_im, B_log_dt, B_Dskip):
    def _A_ref(x, wqkv, wo):
        B, S, D = x.shape
        H = 32; Dh = D // H; W = 256
        qkv = (lambda x, *d: x.transpose(*d))((x @ wqkv).reshape(B, S, 3, H, Dh), 2, 0, 3, 1, 4)
        q, k, v = qkv[0], qkv[1], qkv[2]
        scores = jnp.einsum("bhqd,bhkd->bhqk", q, k) * (Dh ** -0.5)
        idx = jnp.arange(S)
        mask = (idx[:, None] - idx[None, :] >= 0) & (idx[:, None] - idx[None, :] < W)
        scores = jnp.where(mask[None, None], scores, -1e9)
        p = _softmax(scores, axis=-1)
        o = jnp.einsum("bhqk,bhkd->bhqd", p, v)
        return (lambda x, *d: x.transpose(*d))(o, 0, 2, 1, 3).reshape(B, S, D) @ wo

    def _B_ref(u, A_re, A_im, B_re, B_im, C_re, C_im, log_dt, Dskip):
        Bsz, L, D = u.shape
        dt = jnp.exp(log_dt)[:, None]
        A = A_re + 1j * A_im
        Bc = B_re + 1j * B_im
        Cc = C_re + 1j * C_im
        logdA = dt * A
        dB = dt * Bc
        l = (lambda x, dt: x.astype(dt))(jnp.arange(L), A_re.dtype)
        P = jnp.exp(logdA[:, :, None] * l[None, None, :])
        K = jnp.einsum("dn,dnl,dn->dl", Cc, P, dB).real
        L2 = 2 * L
        Kp = jnp.pad(K, ((0, 0), (0, L)))
        up = (lambda x, *d: x.transpose(*d))(u, 0, 2, 1)
        up = jnp.pad(up, ((0, 0), (0, 0), (0, L)))
        Kf = (lambda x, axes=(-2,-1): jnp.fft.rfft2(x.astype(jnp.float32), axes=axes))(Kp[:, None, :], axes=(-2, -1))
        Uf = (lambda x, axes=(-2,-1): jnp.fft.rfft2(x.astype(jnp.float32), axes=axes))(up[:, :, None, :], axes=(-2, -1))
        Yf = Uf * Kf[None, :, :, :]
        y = (lambda x, s, axes=(-2,-1): jnp.fft.irfft2(x, s=s, axes=axes).astype(jnp.bfloat16))(Yf, (1, L2), axes=(-2, -1))[:, :, 0, :L]
        y = (lambda x, *d: x.transpose(*d))(y, 0, 2, 1) + u * Dskip[None, None, :]
        return y

    a = _A_ref(A_x, A_wqkv, A_wo)
    b = _B_ref(B_u, B_A_re, B_A_im, B_B_re, B_B_im, B_C_re, B_C_im, B_log_dt, B_Dskip)
    return jnp.concatenate([a, b], axis=-1)
```

```python
import jax
import jax.numpy as jnp
import numpy as np
from jax.experimental import pallas as pl
from jax.experimental.pallas import tpu as pltpu

S = 2048
D = 512
H, DH, WIN = 32, 16, 256
BQ = 128
NB = S // BQ
PAD = 256
KW = PAD + BQ
NEG = -1e9
HW = 8
NG = H // HW
N = 128
Q = BQ
NC = S // Q
NF = 2 * Q
NACC = 16

_SLOT = {}
for _g in (1, 2, 4, 8):
    for _p in range(NACC):
        _SLOT.setdefault(_g * _p, len(_SLOT))
NPL = len(_SLOT)

bf = jnp.bfloat16
f32 = jnp.float32
i32 = jnp.int32


def _nn(a, b):
    return jnp.dot(a, b, preferred_element_type=f32)


def _nt(a, b):
    return jax.lax.dot_general(a, b, (((1,), (1,)), ((), ())), preferred_element_type=f32)


def _sincos(x):
    k = jnp.floor(x * 0.6366197723675814 + 0.5)
    r = x - k * 1.5703125
    r = r - k * 4.837512969970703125e-4
    r = r - k * 7.54978995489188216e-8
    r2 = r * r
    s = r + r * r2 * (-1.6666654611e-1 + r2 * (8.3321608736e-3 + r2 * (-1.9515295891e-4)))
    c = 1.0 - 0.5 * r2 + r2 * r2 * (4.166664568298827e-2 + r2 * (-1.388731625493765e-3 + r2 * 2.443315711809948e-5))
    q = k.astype(i32)
    swap = (q & 1) == 1
    s_, c_ = jnp.where(swap, c, s), jnp.where(swap, s, c)
    s_ = jnp.where((q & 2) == 2, -s_, s_)
    c_ = jnp.where(((q + 1) & 2) == 2, -c_, c_)
    return s_, c_


def _cmul(ar, ai, br, bi):
    return ar * br - ai * bi, ar * bi + ai * br


def _sel_matrix(g):
    j = jax.lax.broadcasted_iota(i32, (Q, Q), 0)
    p = jax.lax.broadcasted_iota(i32, (Q, Q), 1)
    t2 = 2 * g
    base = (j // t2) * t2
    rem = j - base
    rho = base + jnp.where(rem * 2 <= g, 0, jnp.where(rem * 2 < 3 * g, g, t2))
    return jnp.where(p * g == rho, 1.0, 0.0).astype(bf)


def _dft_consts():
    row = jax.lax.broadcasted_iota(i32, (NF, Q), 0)
    j = jax.lax.broadcasted_iota(i32, (NF, Q), 1)
    k = row & (Q - 1)
    s, c = _sincos(((k * j) & (NF - 1)).astype(f32) * (2.0 * np.pi / NF))
    F = jnp.where(row < Q, c, jnp.where(row == Q, jnp.where((j & 1) == 0, 1.0, -1.0), -s))
    b = jax.lax.broadcasted_iota(i32, (Q, NF), 0)
    col = jax.lax.broadcasted_iota(i32, (Q, NF), 1)
    k2 = col & (Q - 1)
    s2, c2 = _sincos(((k2 * b) & (NF - 1)).astype(f32) * (2.0 * np.pi / NF))
    w = jnp.where(k2 == 0, 1.0 / NF, 2.0 / NF)
    nyq = jnp.where((b & 1) == 0, 1.0, -1.0) * (1.0 / NF)
    Fi = jnp.where(col < Q, c2 * w, jnp.where(col == Q, nyq, -s2 * w))
    return F, Fi


def _kernel(x_hbm, wqkv_hbm, wo_hbm, u_ref, are_ref, aim_ref, bre_ref, bim_ref, cre_ref, cim_ref, ldt_ref, dsk_ref,
            o_ref,
            eye_scr, qt_scr, k_scr, vt_scr, bias_scr, wq_scr, st_scr, ot_scr, wo_scr, wt_scr, x_ref, wqkv_ref, sems,
            tr_scr, ti_scr, v_scr, zm_scr, g_scr, fs_scr, fi_scr, uh_scr, kh_scr, zp_scr, za_scr):
    a = pl.program_id(0)

    @pl.when(a == 0)
    def _init():
        r = jax.lax.broadcasted_iota(i32, (Q, Q), 0)
        c = jax.lax.broadcasted_iota(i32, (Q, Q), 1)
        eye = jnp.where(r == c, 1.0, 0.0).astype(bf)
        eye_scr[...] = eye

        cp_w = pltpu.make_async_copy(wqkv_hbm, wqkv_ref, sems.at[0])
        cp_x = pltpu.make_async_copy(x_hbm, x_ref, sems.at[1])
        cp_o = pltpu.make_async_copy(wo_hbm, wo_scr, sems.at[2])
        cp_w.start()
        cp_x.start()
        cp_o.start()

        def tr(ref):
            return _nt(eye, ref[...])
        dt = jnp.exp(ldt_ref[...].astype(f32)).astype(bf).astype(f32)
        lr = dt * tr(are_ref)
        li = dt * tr(aim_ref)
        cbr, cbi = _cmul(tr(cre_ref), tr(cim_ref), dt * tr(bre_ref), dt * tr(bim_ref))
        v_scr[0] = cbr
        v_scr[1] = cbi

        def anchor(e):
            s, c_ = _sincos(li * float(e))
            mag = jnp.exp(lr * float(e))
            return mag * c_, mag * s

        slot = _SLOT

        def put(e, v):
            tr_scr[slot[e]] = v[0]
            ti_scr[slot[e]] = v[1]

        def mk(e, x, y):
            put(e, _cmul(tr_scr[slot[x]], ti_scr[slot[x]], tr_scr[slot[y]], ti_scr[slot[y]]))

        put(1, anchor(1))
        put(8, anchor(8))
        put(64, anchor(64))
        z128 = anchor(128)
        zm_scr[3, 0] = z128[0]
        zm_scr[3, 1] = z128[1]
        mk(2, 1, 1); mk(3, 2, 1); mk(4, 2, 2); mk(5, 4, 1); mk(6, 4, 2); mk(7, 4, 3)
        for e in range(9, 16):
            mk(e, 8, e - 8)
        mk(16, 8, 8)
        for e in range(18, 32, 2):
            mk(e, 16, e - 16)
        mk(32, 16, 16)
        for e in range(36, 64, 4):
            mk(e, 32, e - 32)
        for e in range(72, 128, 8):
            mk(e, 64, e - 64)
        for gi, e in enumerate((16, 32, 64)):
            zm_scr[gi, 0] = tr_scr[slot[e]]
            zm_scr[gi, 1] = ti_scr[slot[e]]

        F, Fi = _dft_consts()
        fi_scr[...] = Fi.astype(bf)
        fh = F.astype(bf)
        fl = (F - fh.astype(f32)).astype(bf)
        fl2 = (F - fh.astype(f32) - fl.astype(f32)).astype(bf)
        fs_scr[0] = fh
        for gi, g in enumerate((2, 4, 8)):
            sel = _sel_matrix(g)
            fs_scr[gi + 1] = (_nn(fh, sel) + _nn(fl, sel) + _nn(fl2, sel)).astype(bf)
        zp_scr[...] = jnp.zeros(zp_scr.shape, f32)

        cp_w.wait()
        cp_x.wait()
        cp_o.wait()
        wq_scr[...] = jnp.zeros(wq_scr.shape, bf)
        k_scr[0:PAD, :] = jnp.zeros((PAD, D), bf)
        vt_scr[:, 0:PAD] = jnp.zeros((D, PAD), bf)
        for t in range(D // 128):
            rows = slice(t * 128, (t + 1) * 128)
            wt_scr[0, rows, :] = (_nt(eye, wqkv_ref[:, t * 128:(t + 1) * 128]) * 0.25).astype(bf)
            wt_scr[1, rows, :] = _nt(eye, wqkv_ref[:, 2 * D + t * 128: 2 * D + (t + 1) * 128]).astype(bf)

        def project(cb, carry):
            r0 = pl.multiple_of(cb * 512, 512)
            xb = x_ref[pl.ds(r0, 512), :]
            qt_scr[:, pl.ds(r0, 512)] = _nt(wt_scr[0], xb).astype(bf)
            vt_scr[:, pl.ds(PAD + r0, 512)] = _nt(wt_scr[1], xb).astype(bf)
            k_scr[pl.ds(PAD + r0, 512), :] = _nn(xb, wqkv_ref[:, D:2 * D]).astype(bf)
            return carry

        jax.lax.fori_loop(0, S // 512, project, 0)

    @pl.when(a <= 2)
    def _bias():
        r = jax.lax.broadcasted_iota(i32, (KW, BQ), 0)
        c = jax.lax.broadcasted_iota(i32, (KW, BQ), 1)
        diff = c + PAD - r
        valid = (diff >= 0) & (diff < WIN) & (r >= PAD - a * BQ)
        bias_scr[...] = jnp.where(valid, 0.0, NEG).astype(f32)

    q0 = pl.multiple_of(a * BQ, BQ)
    for gi in range(NG):
        for j in range(HW):
            h = gi * HW + j
            rloc = (h % 8) * DH
            wq_scr[gi, rloc:rloc + DH, j * BQ:(j + 1) * BQ] = qt_scr[h * DH:(h + 1) * DH, pl.ds(q0, BQ)]

    def scores(gi):
        g = (gi * HW) // 8
        st_scr[gi] = _nn(k_scr[pl.ds(q0, KW), g * 128:(g + 1) * 128], wq_scr[gi])

    def softmax_pv(gi):
        for j in range(HW):
            r0 = (gi * HW + j) * DH
            for bi, b in enumerate((2, 1, 0)):
                s = st_scr[gi, b * BQ:(b + 1) * BQ, j * BQ:(j + 1) * BQ] + bias_scr[b * BQ:(b + 1) * BQ, :]
                bm = jnp.max(s, axis=0, keepdims=True)
                m_new = bm if bi == 0 else jnp.maximum(m, bm)
                p = jnp.exp(s - m_new)
                ps = jnp.sum(p, axis=0, keepdims=True)
                ob = _nn(vt_scr[r0:r0 + DH, pl.ds(q0 + b * BQ, BQ)], p.astype(bf))
                if bi == 0:
                    acc, l = ob, ps
                else:
                    sc = jnp.exp(m - m_new)
                    acc = acc * sc + ob
                    l = l * sc + ps
                m = m_new
            ot_scr[r0:r0 + DH, :] = (acc / l).astype(bf)

    scores(0)
    for gi in range(NG):
        if gi + 1 < NG:
            scores(gi + 1)
        softmax_pv(gi)
    o_blk = _nt(eye_scr[...], ot_scr[...]).astype(bf)
    o_ref[:, 0:D] = _nn(o_blk, wo_scr[...]).astype(o_ref.dtype)

    lvl = (a >= 2).astype(i32) + (a >= 4).astype(i32) + (a >= 8).astype(i32)
    n_units = jax.lax.shift_right_logical(jnp.int32(Q // NACC), lvl)
    g_scr[...] = jnp.zeros(g_scr.shape, f32)

    def make_unit(lv):
        def unit(p1, carry):
            row = pl.multiple_of(p1 * NACC, NACC)
            for lb in range(D // 128):
                sl = slice(lb * 128, (lb + 1) * 128)
                acc = [None] * NACC
                for nv in range(N // 8):
                    rs = slice(nv * 8, nv * 8 + 8)
                    va = v_scr[0, rs, sl]
                    vb = v_scr[1, rs, sl]
                    for p in range(NACC):
                        if p == 0:
                            t = va
                        else:
                            e = _SLOT[(1 << lv) * p]
                            t = va * tr_scr[e, rs, sl] - vb * ti_scr[e, rs, sl]
                        acc[p] = t if acc[p] is None else acc[p] + t
                g_scr[pl.ds(row, NACC), sl] = jnp.concatenate(
                    [jnp.sum(acc[p], axis=0, keepdims=True) for p in range(NACC)], axis=0)
            nr, ni = _cmul(v_scr[0], v_scr[1], zm_scr[lv, 0], zm_scr[lv, 1])
            v_scr[0] = nr
            v_scr[1] = ni
            return carry
        return unit

    for lv in range(4):
        @pl.when(lvl == lv)
        def _(lv=lv):
            jax.lax.fori_loop(0, (Q // NACC) >> lv, make_unit(lv), 0)

    g_scr[pl.ds(pl.multiple_of(n_units * NACC, NACC), 8), :] = jnp.broadcast_to(
        jnp.sum(v_scr[0], axis=0, keepdims=True), (8, D))
    kh_scr[a] = _nn(fs_scr[lvl], g_scr[0:Q, :].astype(bf))

    ub = u_ref[...]
    uh_scr[a] = _nn(fs_scr[0], ub)

    RT = 32
    row0 = jax.lax.broadcasted_iota(i32, (RT, 128), 0) == 0

    def conv_block(cs, first=False):
        for rt in range(Q // RT):
            rs = slice(rt * RT, (rt + 1) * RT)
            rs2 = slice(Q + rt * RT, Q + (rt + 1) * RT)
            for lb in range(D // 128):
                sl = slice(lb * 128, (lb + 1) * 128)
                zr = None if first else za_scr[rs, sl]
                zi = None if first else za_scr[rs2, sl]
                for c_ in cs:
                    kr = kh_scr[a - c_, rs, sl]; ki = kh_scr[a - c_, rs2, sl]
                    ur = uh_scr[c_, rs, sl]; ui = uh_scr[c_, rs2, sl]
                    aa = ki * ui
                    if rt == 0:
                        pr = kr * ur - jnp.where(row0, 0.0, aa)
                        pi = jnp.where(row0, aa, kr * ui + ki * ur)
                    else:
                        pr = kr * ur - aa
                        pi = kr * ui + ki * ur
                    zr = pr if zr is None else zr + pr
                    zi = pi if zi is None else zi + pi
                za_scr[rs, sl] = zr
                za_scr[rs2, sl] = zi

    odd = a & 1

    @pl.when(odd == 0)
    def _():
        conv_block((0,), first=True)

    @pl.when(odd == 1)
    def _():
        conv_block((0, 1), first=True)

    def conv_pair(t, carry):
        c = 1 + odd + 2 * t
        conv_block((c, c + 1))
        return carry

    jax.lax.fori_loop(0, a // 2, conv_pair, 0)

    sgn = jnp.where((jax.lax.broadcasted_iota(i32, (NF, D), 0) & 1) == 0, 1.0, -1.0)
    z = za_scr[...]
    w = z + sgn * zp_scr[...]
    zp_scr[...] = z
    y = _nn(fi_scr[...], w.astype(bf)).astype(bf)
    o_ref[:, D:2 * D] = (y + ub * dsk_ref[...]).astype(o_ref.dtype)


@jax.jit
def pallas_concat_heads__sliding_block__ssm_conv_s4__prompt_kernel(
    A_x: jax.Array,
    A_wqkv: jax.Array,
    A_wo: jax.Array,
    B_u: jax.Array,
    B_A_re: jax.Array,
    B_A_im: jax.Array,
    B_B_re: jax.Array,
    B_B_im: jax.Array,
    B_C_re: jax.Array,
    B_C_im: jax.Array,
    B_log_dt: jax.Array,
    B_Dskip: jax.Array,
):
    def full(shape):
        return pl.BlockSpec(shape, lambda i: tuple(0 for _ in shape))

    out = pl.pallas_call(
        _kernel,
        grid=(NB,),
        in_specs=[pl.BlockSpec(memory_space=pl.ANY)] * 3 + [
                  pl.BlockSpec((Q, D), lambda i: (i, 0))]
                 + [full((D, N))] * 6 + [full((1, D)), full((1, D))],
        out_specs=pl.BlockSpec((BQ, 2 * D), lambda i: (i, 0)),
        out_shape=jax.ShapeDtypeStruct((S, 2 * D), bf),
        scratch_shapes=[
            pltpu.VMEM((BQ, BQ), bf),
            pltpu.VMEM((D, S), bf),
            pltpu.VMEM((S + PAD, D), bf),
            pltpu.VMEM((D, S + PAD), bf),
            pltpu.VMEM((KW, BQ), f32),
            pltpu.VMEM((NG, 128, HW * BQ), bf),
            pltpu.VMEM((NG, KW, HW * BQ), f32),
            pltpu.VMEM((D, BQ), bf),
            pltpu.VMEM((D, D), bf),
            pltpu.VMEM((2, D, D), bf),
            pltpu.VMEM((S, D), bf),
            pltpu.VMEM((D, 3 * D), bf),
            pltpu.SemaphoreType.DMA((3,)),
            pltpu.VMEM((NPL, N, D), f32),
            pltpu.VMEM((NPL, N, D), f32),
            pltpu.VMEM((2, N, D), f32),
            pltpu.VMEM((4, 2, N, D), f32),
            pltpu.VMEM((Q + 8, D), f32),
            pltpu.VMEM((4, NF, Q), bf),
            pltpu.VMEM((Q, NF), bf),
            pltpu.VMEM((NC, NF, D), f32),
            pltpu.VMEM((NC, NF, D), f32),
            pltpu.VMEM((NF, D), f32),
            pltpu.VMEM((NF, D), f32),
        ],
        compiler_params=pltpu.CompilerParams(
            dimension_semantics=("arbitrary",), vmem_limit_bytes=112 * 1024 * 1024),
    )(A_x.reshape(S, D), A_wqkv, A_wo, B_u.reshape(S, D), B_A_re, B_A_im, B_B_re, B_B_im, B_C_re, B_C_im,
      B_log_dt.reshape(1, D), B_Dskip.reshape(1, D))
    return out.reshape(1, S, 2 * D)
```
